```python
import os as _os
_os.environ.setdefault("JAX_PLATFORMS", "cpu")
import jax
import jax.numpy as jnp

def _softmax(x, axis=-1):
    return jax.nn.softmax(x, axis=axis)
def _gelu(x):
    return jax.nn.gelu(x, approximate=True)
def _silu(x):
    return jax.nn.silu(x)
def _sigmoid(x):
    return jax.nn.sigmoid(x)
def _layernorm(x, axis=-1, eps=1e-5):
    m = jnp.mean(x, axis=axis, keepdims=True)
    v = jnp.var(x, axis=axis, keepdims=True)
    return (x - m) / jnp.sqrt(v + eps)
def _scatter_add(tgt, idx, src, axis=0):
    return tgt.at[idx].add(src)
def _segment_sum(src, seg, n):
    return jax.ops.segment_sum(src, seg, n)
class _Rng:
    def __init__(self, key):
        self._k = key
    def _next(self):
        self._k, sub = jax.random.split(self._k)
        return sub
    def normal(self, shape):
        return jax.random.normal(self._next(), shape, dtype=jnp.bfloat16)
    def randint(self, lo, hi, shape):
        return jax.random.randint(self._next(), shape, lo, hi, dtype=jnp.int32)
    def uniform(self, shape, lo=0.0, hi=1.0):
        return jax.random.uniform(self._next(), shape, jnp.bfloat16, lo, hi)
    def permutation(self, n):
        return jax.random.permutation(self._next(), n)


kernel_name = 'standalone__gqa_block_cached__near_ridge'

def setup_inputs():
    _rng = _Rng(jax.random.key(int.from_bytes(__import__("os").urandom(4), "little")))
    _w = (lambda a: (lambda t: t.astype(jnp.bfloat16) if jnp.issubdtype(t.dtype, jnp.floating) else t)(jnp.asarray(a)))
    B, Sq, D = 8, 96, 448
    Hq, Hkv, Sk, Dh = 16, 8, 2048, 256
    assert Hq % Hkv == 0, (Hq, Hkv)
    return {
        "x": _w((lambda *s: _rng.normal(s) * 0.8)(B, Sq, D)),
        "k_cache": _w((lambda *s: _rng.normal(s) * 0.8)(B, Hkv, Sk, Dh)),
        "v_cache": _w((lambda *s: _rng.normal(s) * 0.05)(B, Hkv, Sk, Dh)),
        "wq": _w((lambda *s: _rng.normal(s) * 0.8)(D, Hq * Dh) * (D ** -0.5)),
        "wo": _w((lambda *s: _rng.normal(s) * 0.05)(Hq * Dh, D) * ((Hq * Dh) ** -0.5)),
    }

def reference(x, k_cache, v_cache, wq, wo):
    B, Sq, D = x.shape
    Hq, Dh = 16, 256
    Hkv = k_cache.shape[1]
    rep = Hq // Hkv
    q = (lambda x, *d: x.transpose(*d))((x @ wq).reshape(B, Sq, Hq, Dh), 0, 2, 1, 3)
    k = jnp.repeat(k_cache, rep, axis=1)
    v = jnp.repeat(v_cache, rep, axis=1)
    scores = jnp.einsum("bhqd,bhkd->bhqk", q, k) * (Dh ** -0.5)
    p = _softmax(scores, axis=-1)
    o = jnp.einsum("bhqk,bhkd->bhqd", p, v)
    return (lambda x, *d: x.transpose(*d))(o, 0, 2, 1, 3).reshape(B, Sq, Hq * Dh) @ wo
```

```python
import functools
import jax
import jax.numpy as jnp
import numpy as np
from jax.experimental import pallas as pl
from jax.experimental.pallas import tpu as pltpu

B, SQ, D = 8, 96, 448
HQ, HKV, SK, DH = 16, 8, 2048, 256
REP = HQ // HKV
T = B * HKV
M = REP * SQ
LOG2E = 1.4426950408889634
QSCALE = float(DH ** -0.5 * LOG2E)
FLAGS = {"XLA_TPU_FORCE_LP_LLO_SCHEDULER": True}
NT_DIMS = (((1,), (1,)), ((), ()))


def make_kernel(NB=4, U=2, nodma=False, PC=8, pattern="qkvo", pk=0, pv=0, pw=0, po=0):
    assert NB % U == 0 and B % U == 0
    def _kernel(x_hbm, wq_hbm, wo_hbm, k_hbm, v_hbm, o_hbm,
                x_v, wq_v, wo_v, k_v, v_v, q_a, q_b, s_a, s_b, o_a, o_b, acc, out_v,
                sem_x, sem_wq, sem_wo, sem_k, sem_v, sem_o):
        Q = (q_a, q_b); S = (s_a, s_b); O = (o_a, o_b)
        static = lambda t: isinstance(t, int)

        def when(c):
            if isinstance(c, (bool, np.bool_)):
                return (lambda f: f() if c else None)
            return pl.when(c)

        def k_copy(t):
            slot = t % NB
            return pltpu.make_async_copy(k_hbm.at[t % B, t // B], k_v.at[slot], sem_k.at[slot])

        def v_copy(t):
            slot = t % NB
            return pltpu.make_async_copy(v_hbm.at[t % B, t // B], v_v.at[slot], sem_v.at[slot])

        def wcol(h):
            return pl.ds(h * (REP * DH), REP * DH) if static(h) else pl.ds(pl.multiple_of(h * (REP * DH), REP * DH), REP * DH)

        def wq_copy(h):
            return pltpu.make_async_copy(wq_hbm.at[:, wcol(h)], wq_v.at[h], sem_wq.at[h])

        def wo_copy(h):
            return pltpu.make_async_copy(wo_hbm.at[:, wcol(h)], wo_v.at[h], sem_wo.at[h])

        def out_copy(b):
            return pltpu.make_async_copy(out_v.at[b], o_hbm.at[b], sem_o.at[b])

        x_copy = pltpu.make_async_copy(x_hbm, x_v, sem_x.at[0])

        def qproj(t, par):
            q = jnp.dot(x_v[t % B], wq_v[t // B], preferred_element_type=jnp.float32) * QSCALE
            q = q.astype(jnp.bfloat16)
            for r in range(REP):
                Q[par][r * SQ:(r + 1) * SQ, :] = q[:, r * DH:(r + 1) * DH]

        def qk(t, par):
            S[par][...] = jax.lax.dot_general(Q[par][...], k_v[t % NB], NT_DIMS, preferred_element_type=jnp.float32)

        def smpv(t, par):
            n = SK // PC
            m = jnp.max(S[par][...], axis=-1, keepdims=True)
            o = None
            lacc = None
            for c in range(PC):
                p = jnp.exp2(S[par][:, c * n:(c + 1) * n] - m)
                pl_ = p[:, 0:128]
                for j in range(1, n // 128):
                    pl_ = pl_ + p[:, j * 128:(j + 1) * 128]
                lacc = pl_ if lacc is None else lacc + pl_
                part = jnp.dot(p.astype(jnp.bfloat16), v_v[t % NB, c * n:(c + 1) * n, :], preferred_element_type=jnp.float32)
                o = part if o is None else o + part
            l = jnp.sum(lacc, axis=-1, keepdims=True)
            o = (o * (1.0 / l)).astype(jnp.bfloat16)
            for r in range(REP):
                O[par][:, r * DH:(r + 1) * DH] = o[r * SQ:(r + 1) * SQ, :]

        def oproj(t, par):
            b = t % B
            new = acc[b] + jax.lax.dot_general(O[par][...], wo_v[t // B], NT_DIMS, preferred_element_type=jnp.float32)
            acc[b] = new
            out_v[b] = new.astype(out_v.dtype)

        def compute(t, par):
            ok = lambda s: (not static(s)) or (0 <= s < T)
            for ch in pattern:
                if ch == "q" and ok(t + 2): qproj(t + 2, par)
                if ch == "k" and ok(t + 1): qk(t + 1, 1 - par)
                if ch == "v" and ok(t): smpv(t, par)
                if ch == "o" and ok(t - 1): oproj(t - 1, 1 - par)

        def dma_section(t0):
            t1 = t0 + U
            for j in range(U):
                kt = t0 + 1 + j + NB
                vt = t0 + j + NB
                if nodma: continue
                @when(kt < T)
                def _():
                    k_copy(kt).start(priority=pk)
                @when(vt < T)
                def _():
                    v_copy(vt).start(priority=pv)
            b1 = t1 % B
            h1 = t1 // B
            hs = (lambda h: h) if static(h1) else (lambda h: jnp.minimum(h, HKV - 1))
            andf = (lambda a, b: a and b) if static(t0) else jnp.logical_and
            @when(andf(b1 == 0, h1 + 1 < HKV))
            def _():
                wo_copy(hs(h1 + 1)).start(priority=pw)
            @when(andf(b1 == 0, h1 + 2 < HKV))
            def _():
                wq_copy(hs(h1 + 2)).start(priority=pw)
            for j in range(U):
                to = t0 - 1 + j
                @when(to >= max(T - B, 0))
                def _():
                    out_copy(to % B).start(priority=po)
            for j in range(U):
                tq = t1 + 2 + j
                @when(andf(tq % B == 0, tq < T))
                def _():
                    wq_copy(hs(tq // B)).wait()
                to = t1 - 1 + j
                @when(andf(to % B == 0, to < T))
                def _():
                    wo_copy(hs(to // B)).wait()
            if not nodma:
                for j in range(U):
                    kt = t1 + 1 + j
                    vt = t1 + j
                    @when(kt < T)
                    def _():
                        k_copy(kt).wait()
                    @when(vt < T)
                    def _():
                        v_copy(vt).wait()

        x_copy.start()
        wq_copy(0).start()
        k_copy(0).start()
        for j in range(1, NB - U + 1):
            k_copy(j).start()
            if j - 1 < NB - U: v_copy(j - 1).start()
            if j == 1: wo_copy(0).start()
        wq_copy(1).start()
        acc[...] = jnp.zeros_like(acc)
        x_copy.wait()
        wq_copy(0).wait()
        qproj(0, 0)
        qproj(1, 1)
        k_copy(0).wait()
        qk(0, 0)
        if nodma:
            for j in range(1, NB - U + 1): k_copy(j).wait()
            for j in range(0, NB - U): v_copy(j).wait()

        G = max(U, 2)
        def superg(t0):
            for g in range(G // U):
                for j in range(U):
                    compute(t0 + g * U + j, (g * U + j) % 2)
                dma_section(t0 + g * U)
        dma_section(-U)
        superg(0)
        last_dyn = (T - 2 - G) // G
        def body(i, _):
            superg(i * G)
            return 0
        jax.lax.fori_loop(1, last_dyn + 1, body, 0)
        for g in range(last_dyn + 1, T // G):
            superg(g * G)
        oproj(T - 1, (T - 1) % 2)
        out_copy(B - 1).start()
        for b in range(B):
            out_copy(b).wait()

    return _kernel


def build(NB=4, U=2, nodma=False, nobc=True, **kw):
    @jax.jit
    def kernel(x, k_cache, v_cache, wq, wo):
        hbm = pl.BlockSpec(memory_space=pltpu.MemorySpace.HBM)
        bf, f32 = jnp.bfloat16, jnp.float32
        return pl.pallas_call(
            make_kernel(NB, U, nodma, **kw),
            in_specs=[hbm] * 5,
            out_specs=hbm,
            out_shape=jax.ShapeDtypeStruct((B, SQ, D), bf),
            scratch_shapes=[
                pltpu.VMEM((B, SQ, D), bf),
                pltpu.VMEM((HKV, D, REP * DH), bf),
                pltpu.VMEM((HKV, D, REP * DH), bf),
                pltpu.VMEM((NB, SK, DH), bf),
                pltpu.VMEM((NB, SK, DH), bf),
                pltpu.VMEM((M, DH), bf), pltpu.VMEM((M, DH), bf),
                pltpu.VMEM((M, SK), f32), pltpu.VMEM((M, SK), f32),
                pltpu.VMEM((SQ, REP * DH), bf), pltpu.VMEM((SQ, REP * DH), bf),
                pltpu.VMEM((B, SQ, D), f32),
                pltpu.VMEM((B, SQ, D), bf),
                pltpu.SemaphoreType.DMA((1,)),
                pltpu.SemaphoreType.DMA((HKV,)),
                pltpu.SemaphoreType.DMA((HKV,)),
                pltpu.SemaphoreType.DMA((NB,)),
                pltpu.SemaphoreType.DMA((NB,)),
                pltpu.SemaphoreType.DMA((B,)),
            ],
            compiler_params=pltpu.CompilerParams(vmem_limit_bytes=100 * 2**20, disable_bounds_checks=nobc, flags=FLAGS),
        )(x, wq, wo.T, k_cache, v_cache)
    return kernel


pallas_standalone__gqa_block_cached__near_ridge_kernel = build(3, 1)
```

```python
import functools
import jax
import jax.numpy as jnp
import numpy as np
from jax.experimental import pallas as pl
from jax.experimental.pallas import tpu as pltpu

B, SQ, D = 8, 96, 448
HQ, HKV, SK, DH = 16, 8, 2048, 256
REP = HQ // HKV
T = B * HKV
M = REP * SQ
LOG2E = 1.4426950408889634
QSCALE = float(DH ** -0.5 * LOG2E)
FLAGS = {"XLA_TPU_FORCE_LP_LLO_SCHEDULER": True}
NT_DIMS = (((1,), (1,)), ((), ()))


def make_kernel(NB=3, PC=8, BB=2, maxmode="B", split=True, pk=0, pv=0, WB=0, tail=0):
    def _kernel(x_hbm, wq_hbm, wo_hbm, k_hbm, v_hbm, o_hbm,
                x_v, wq_v, wo_v, k_v, v_v, q_all, s_a, s_b, o_a, o_b, acc, out_v, m_a, m_b,
                sem_x, sem_wq, sem_wo, sem_k, sem_v, sem_o):
        S = (s_a, s_b); O = (o_a, o_b); MX = (m_a, m_b)
        static = lambda t: isinstance(t, int)

        def when(c):
            if isinstance(c, (bool, np.bool_)):
                return (lambda f: f() if c else None)
            return pl.when(c)

        def k_copy(t):
            return pltpu.make_async_copy(k_hbm.at[t % B, t // B], k_v.at[t % NB], sem_k.at[t % NB])

        def v_copy(t):
            return pltpu.make_async_copy(v_hbm.at[t % B, t // B], v_v.at[t % NB], sem_v.at[t % NB])

        def wcol(h):
            return pl.ds(h * (REP * DH), REP * DH) if static(h) else pl.ds(pl.multiple_of(h * (REP * DH), REP * DH), REP * DH)

        def wq_copy(h):
            return pltpu.make_async_copy(wq_hbm.at[:, wcol(h)], wq_v.at[h], sem_wq.at[h])

        def wo_copy(h):
            return pltpu.make_async_copy(wo_hbm.at[:, wcol(h)], wo_v.at[h], sem_wo.at[h])

        def out_copy(b):
            return pltpu.make_async_copy(out_v.at[b], o_hbm.at[b], sem_o.at[b])

        x_copy = pltpu.make_async_copy(x_hbm, x_v, sem_x.at[0])

        def qburst(h):
            q = jnp.dot(x_v[...], wq_v[h], preferred_element_type=jnp.float32) * QSCALE
            q = q.astype(jnp.bfloat16)
            for bb in range(B):
                for r in range(REP):
                    q_all[h % 2, bb, r * SQ:(r + 1) * SQ, :] = q[bb * SQ:(bb + 1) * SQ, r * DH:(r + 1) * DH]

        def qk(t, par):
            S[par][...] = jax.lax.dot_general(q_all[(t // B) % 2, t % B], k_v[t % NB], NT_DIMS, preferred_element_type=jnp.float32)

        def rowmax(par):
            MX[par][...] = jnp.broadcast_to(jnp.max(S[par][...], axis=-1, keepdims=True), (M, 128))

        def smpv(t, par):
            n = SK // PC
            if maxmode == "B":
                m = jnp.max(S[par][...], axis=-1, keepdims=True)
            else:
                m = jnp.concatenate([MX[par][...]] * (n // 128), axis=1)
            o = None
            lacc = None
            for c in range(PC):
                p = jnp.exp2(S[par][:, c * n:(c + 1) * n] - m)
                pl_ = p[:, 0:128]
                for j in range(1, n // 128):
                    pl_ = pl_ + p[:, j * 128:(j + 1) * 128]
                lacc = pl_ if lacc is None else lacc + pl_
                part = jnp.dot(p.astype(jnp.bfloat16), v_v[t % NB, c * n:(c + 1) * n, :], preferred_element_type=jnp.float32)
                o = part if o is None else o + part
            l = jnp.sum(lacc, axis=-1, keepdims=True)
            o = (o * (1.0 / l)).astype(jnp.bfloat16)
            for r in range(REP):
                O[par][:, r * DH:(r + 1) * DH] = o[r * SQ:(r + 1) * SQ, :]

        def oproj(t, par):
            b = t % B
            h = t // B if static(t) else jnp.maximum(t, 0) // B
            new = acc[b] + jax.lax.dot_general(O[par][...], wo_v[h], NT_DIMS, preferred_element_type=jnp.float32)
            acc[b] = new
            out_v[b] = new.astype(out_v.dtype)

        def step(t, par):
            b = t % B
            h = t // B
            st = static(t)
            andf = (lambda a, c: a and c) if st else jnp.logical_and
            hs = (lambda x: x) if st else (lambda x: jnp.minimum(x, HKV - 1))
            has_k = (t + 1 < T) if st else True
            if has_k: k_copy(t + 1).wait()
            early = (not split) or (st and not has_k and tail >= 1)
            if early: v_copy(t).wait()
            if maxmode == "A0": rowmax(par)
            if has_k: qk(t + 1, 1 - par)
            if maxmode == "A1" and has_k: rowmax(1 - par)
            oproj(t - 1, 1 - par)
            if has_k:
                @when(t + 1 + NB < T)
                def _():
                    k_copy(t + 1 + NB).start(priority=pk)
            @when(t - 1 >= T - B)
            def _():
                out_copy((t - 1) % B).start()
            if not early: v_copy(t).wait()
            smpv(t, par)
            @when(t + NB < T)
            def _():
                v_copy(t + NB).start(priority=pv)
            if par == 0:
                @when(andf(b == WB, h + 1 < HKV))
                def _():
                    wo_copy(hs(h + 1)).start()

                @when(andf(b == WB, h + 2 < HKV))
                def _():
                    wq_copy(hs(h + 2)).start()

                @when(andf(b == BB, h + 1 < HKV))
                def _():
                    wq_copy(hs(h + 1)).wait()
                    qburst(hs(h + 1))

                @when(andf(b == B - 2, h + 1 < HKV))
                def _():
                    wo_copy(hs(h + 1)).wait()

        x_copy.start()
        wq_copy(0).start()
        k_copy(0).start()
        wo_copy(0).start()
        for j in range(1, NB):
            k_copy(j).start()
            v_copy(j - 1).start()
        wq_copy(1).start()
        acc[...] = jnp.zeros_like(acc)
        o_b[...] = jnp.zeros_like(o_b)
        x_copy.wait()
        wq_copy(0).wait()
        qburst(0)
        k_copy(0).wait()
        qk(0, 0)
        if maxmode == "A1": rowmax(0)
        k_copy(NB).start()
        v_copy(NB - 1).start()
        wo_copy(0).wait()

        def body(i, _):
            step(2 * i, 0)
            step(2 * i + 1, 1)
            return 0
        jax.lax.fori_loop(0, T // 2 - 1, body, 0)
        step(T - 2, 0)
        step(T - 1, 1)
        oproj(T - 1, 1)
        out_copy(B - 1).start()
        for b in range(B):
            out_copy(b).wait()

    return _kernel


def build(NB=3, **kw):
    @jax.jit
    def kernel(x, k_cache, v_cache, wq, wo):
        hbm = pl.BlockSpec(memory_space=pltpu.MemorySpace.HBM)
        bf, f32 = jnp.bfloat16, jnp.float32
        return pl.pallas_call(
            make_kernel(NB, **kw),
            in_specs=[hbm] * 5,
            out_specs=hbm,
            out_shape=jax.ShapeDtypeStruct((B, SQ, D), bf),
            scratch_shapes=[
                pltpu.VMEM((B * SQ, D), bf),
                pltpu.VMEM((HKV, D, REP * DH), bf),
                pltpu.VMEM((HKV, D, REP * DH), bf),
                pltpu.VMEM((NB, SK, DH), bf),
                pltpu.VMEM((NB, SK, DH), bf),
                pltpu.VMEM((2, B, M, DH), bf),
                pltpu.VMEM((M, SK), f32), pltpu.VMEM((M, SK), f32),
                pltpu.VMEM((SQ, REP * DH), bf), pltpu.VMEM((SQ, REP * DH), bf),
                pltpu.VMEM((B, SQ, D), f32),
                pltpu.VMEM((B, SQ, D), bf),
                pltpu.VMEM((M, 128), f32), pltpu.VMEM((M, 128), f32),
                pltpu.SemaphoreType.DMA((1,)),
                pltpu.SemaphoreType.DMA((HKV,)),
                pltpu.SemaphoreType.DMA((HKV,)),
                pltpu.SemaphoreType.DMA((NB,)),
                pltpu.SemaphoreType.DMA((NB,)),
                pltpu.SemaphoreType.DMA((B,)),
            ],
            compiler_params=pltpu.CompilerParams(vmem_limit_bytes=100 * 2**20, disable_bounds_checks=True, flags=FLAGS),
        )(x.reshape(B * SQ, D), wq, wo.T, k_cache, v_cache)
    return kernel


pallas_standalone__gqa_block_cached__near_ridge_kernel = build(4, BB=0, maxmode="A1")
```
